```python
import jax
import jax.numpy as jnp

def _softmax(x, axis=-1):
    return jax.nn.softmax(x, axis=axis)

def _gelu(x):
    return jax.nn.gelu(x, approximate=True)

def _silu(x):
    return jax.nn.silu(x)

def _sigmoid(x):
    return jax.nn.sigmoid(x)

def _layernorm(x, axis=-1, eps=1e-05):
    m = jnp.mean(x, axis=axis, keepdims=True)
    v = jnp.var(x, axis=axis, keepdims=True)
    return (x - m) / jnp.sqrt(v + eps)

def _scatter_add(tgt, idx, src, axis=0):
    return tgt.at[idx].add(src)

def _segment_sum(src, seg, n):
    return jax.ops.segment_sum(src, seg, n)

class _Rng:

    def __init__(self, key):
        self._k = key

    def _next(self):
        self._k, sub = jax.random.split(self._k)
        return sub

    def normal(self, shape):
        return jax.random.normal(self._next(), shape, dtype=jnp.bfloat16)

    def randint(self, lo, hi, shape):
        return jax.random.randint(self._next(), shape, lo, hi, dtype=jnp.int32)

    def uniform(self, shape, lo=0.0, hi=1.0):
        return jax.random.uniform(self._next(), shape, jnp.bfloat16, lo, hi)

    def permutation(self, n):
        return jax.random.permutation(self._next(), n)
kernel_name = 'adaLN_cond__ssm_conv_h3__dense_activation_gelu__prompt'

def setup_inputs():
    _rng = _Rng(jax.random.key(int.from_bytes(__import__("os").urandom(4), "little")))
    _w = lambda a: (lambda t: t.astype(jnp.bfloat16) if jnp.issubdtype(t.dtype, jnp.floating) else t)(jnp.asarray(a))

    def _A_setup():
        B, S, D = (1, 2048, 640)
        ks = 4
        return {'q': _w((lambda *s: _rng.normal(s) * 0.05)(B, S, D)), 'k': _w((lambda *s: _rng.normal(s) * 0.05)(B, S, D)), 'v': _w((lambda *s: _rng.normal(s) * 0.05)(B, S, D)), 'shift_k': _w((lambda *s: _rng.normal(s) * 0.05)(D, ks) * 0.5), 'ssm_k': _w((lambda *s: _rng.normal(s) * 0.05)(D, S) * (1.0 / S ** 0.5)), 'ssm_D': _w((lambda *s: _rng.normal(s) * 0.05)(D))}
    _A_in = _A_setup()

    def _B_setup():
        B, S, D, F = (1, 2048, 640, 1728)
        return {'x': _w((lambda *s: _rng.normal(s) * 0.05)(B, S, D)), 'w1': _w((lambda *s: _rng.normal(s) * 0.05)(D, F) * D ** (-0.5)), 'b1': _w((lambda *s: _rng.normal(s) * 0.05)(F) * 0.01), 'w2': _w((lambda *s: _rng.normal(s) * 0.05)(F, D) * F ** (-0.5)), 'b2': _w((lambda *s: _rng.normal(s) * 0.05)(D) * 0.01)}
    _B_in = _B_setup()
    return {'A_q': _A_in['q'], 'A_k': _A_in['k'], 'A_v': _A_in['v'], 'A_shift_k': _A_in['shift_k'], 'A_ssm_k': _A_in['ssm_k'], 'A_ssm_D': _A_in['ssm_D'], 'B_x': _B_in['x'], 'B_w1': _B_in['w1'], 'B_b1': _B_in['b1'], 'B_w2': _B_in['w2'], 'B_b2': _B_in['b2'], 'c': _w((lambda *s: _rng.normal(s) * 0.05)(1, 640)), 'w_mod': _w((lambda *s: _rng.normal(s) * 0.05)(640, 6 * 640) * 640 ** (-0.5))}

def reference(A_q, A_k, A_v, A_shift_k, A_ssm_k, A_ssm_D, B_x, B_w1, B_b1, B_w2, B_b2, c, w_mod):

    def _A_ref(q, k, v, shift_k, ssm_k, ssm_D):
        B, S, D = q.shape
        ks = shift_k.shape[-1]
        k_pad = jnp.pad(k, ((0, 0), (ks - 1, 0), (0, 0)))
        k_shift = jnp.zeros_like(k)
        for t in range(ks):
            k_shift = k_shift + k_pad[:, t:t + S, :] * shift_k[:, ks - 1 - t][None, None, :]
        kv = k_shift * v
        L = 2 * S
        kv_pad = jnp.pad(kv, ((0, 0), (0, S), (0, 0)))
        kf_pad = jnp.pad(ssm_k, ((0, 0), (0, S)))
        kv_f = (lambda x, axes=(-2, -1): jnp.fft.rfft2(x.astype(jnp.float32), axes=axes))(kv_pad[:, None, :, :], axes=(1, 2))
        kf_f = (lambda x, axes=(-2, -1): jnp.fft.rfft2(x.astype(jnp.float32), axes=axes))(kf_pad[:, None, :], axes=(1, 2))
        kf_f = (lambda x, *d: x.transpose(*d))(kf_f, 1, 2, 0)
        y_f = kv_f * kf_f[None, :, :, :]
        y = (lambda x, s, axes=(-2, -1): jnp.fft.irfft2(x, s=s, axes=axes).astype(jnp.bfloat16))(y_f, (1, L), axes=(1, 2))[:, 0, :S, :]
        y = y + kv * ssm_D[None, None, :]
        return q * y

    def _B_ref(x, w1, b1, w2, b2):
        h = jnp.einsum('bsd,df->bsf', x, w1) + b1
        h = _gelu(h)
        return jnp.einsum('bsf,fd->bsd', h, w2) + b2
    x = A_q
    mod = (_silu(c) @ w_mod).reshape(c.shape[0], 6, 1, -1)
    sa, ca, ga, sb, cb, gb = (mod[:, 0].copy(), mod[:, 1].copy(), mod[:, 2].copy(), mod[:, 3].copy(), mod[:, 4].copy(), mod[:, 5].copy())
    h = _layernorm(x, axis=-1) * (1 + ca) + sa
    x = x + ga * _A_ref(h, A_k, A_v, A_shift_k, A_ssm_k, A_ssm_D)
    h = _layernorm(x, axis=-1) * (1 + cb) + sb
    x = x + gb * _B_ref(h, B_w1, B_b1, B_w2, B_b2)
    return x
```

```python
import numpy as np
import jax
import jax.numpy as jnp
from jax import lax
import jax.experimental.pallas as pl
import jax.experimental.pallas.tpu as pltpu

S, D, F = 2048, 640, 1728
NT = D // 128
BM, SM = 512, 256
FS = (0, 896, 1728)
U1, U2, U3 = 32, 32, 32


def _dft_consts():
    N = 4096
    n1 = np.arange(32)[None, :]
    j = np.arange(32)[:, None]
    a = 2 * np.pi * n1 * j / 64
    f1 = np.concatenate([np.cos(a), -np.sin(a)], 0)
    f1[32] = (-1.0) ** n1[0]
    n2 = np.arange(64)[None, :]
    k2 = np.arange(64)[:, None]
    G = np.zeros((32, 128, 128))
    H = np.zeros((32, 128, 128))
    for jj in range(1, 32):
        th = 2 * np.pi * ((n2 * (jj + 64 * k2)) % N) / N
        c, s = np.cos(th), np.sin(th)
        G[jj, :64, 0::2], G[jj, :64, 1::2] = c, s
        G[jj, 64:, 0::2], G[jj, 64:, 1::2] = -s, c
        H[jj, :64, :64], H[jj, :64, 64:] = c.T, -s.T
        H[jj, 64:, :64], H[jj, 64:, 64:] = s.T, c.T
    m = np.arange(32)[:, None]
    t0 = 2 * np.pi * ((n2 * m) % 64) / 64
    t1 = 2 * np.pi * ((n2 * (32 + 64 * m)) % N) / N
    r0, i0 = np.cos(t0), -np.sin(t0)
    i0[0] = (-1.0) ** n2[0]
    G[0, 0:32, 0::2], G[0, 64:96, 0::2] = r0, i0
    G[0, 32:64, 1::2], G[0, 96:128, 1::2] = np.cos(t1), -np.sin(t1)
    w = np.full((32, 1), 2.0)
    w[0] = 1.0
    H[0, :64, 0:32], H[0, :64, 64:96] = (w * r0).T, (w * i0).T
    H[0, 64:, 32:64], H[0, 64:, 96:128] = 2 * np.cos(t1).T, -2 * np.sin(t1).T
    a = a.T
    fi = np.zeros((32, 64))
    fi[:, 0::2], fi[:, 1::2] = 2 * np.cos(a), -2 * np.sin(a)
    fi[:, 0] = 1.0
    fi[:, 1] = (-1.0) ** np.arange(32)
    fi /= N
    bf = jnp.bfloat16
    return f1.astype(bf), G.astype(bf), H.astype(bf), fi.astype(bf)


_F1, _G, _H, _FI = _dft_consts()
f32, bf16, u32 = jnp.float32, jnp.bfloat16, jnp.uint32


def _unpack(u):
    lo = pltpu.bitcast(u << 16, f32)
    hi = pltpu.bitcast(u & jnp.uint32(0xFFFF0000), f32)
    return lo, hi


def _pack(lo, hi):
    a = pltpu.bitcast(lo.astype(bf16).astype(f32), u32) >> 16
    b = pltpu.bitcast(hi.astype(bf16).astype(f32), u32)
    return a | b


def _dot(a, b):
    return jnp.dot(a, b, preferred_element_type=f32)


def _ln(x):
    m = jnp.mean(x, axis=-1, keepdims=True)
    xc = x - m
    v = jnp.mean(xc * xc, axis=-1, keepdims=True)
    return xc * lax.rsqrt(v + 1e-5)


def _kernel(q_ref, sk_ref, dd_ref, b1_ref, b2_ref, c_ref, f1_ref, fi_ref,
            k_hbm, v_hbm, s_hbm, w1_hbm, w2_hbm, wm_hbm, g_hbm, h_hbm,
            o_ref,
            kb, vb, sb, st, w1, w2, wm, gm, hm, a_kv, a_k, bsc, kvs, y, mod, dds, sems):
    step = pl.program_id(0)

    def tile_copies(t):
        cs = pl.ds(pl.multiple_of(t * 128, 128), 128)
        return (pltpu.make_async_copy(k_hbm.at[:, cs], kb.at[t], sems.at[3 * t]),
                pltpu.make_async_copy(v_hbm.at[:, cs], vb.at[t], sems.at[3 * t + 1]),
                pltpu.make_async_copy(s_hbm.at[cs, :], sb.at[t], sems.at[3 * t + 2]))

    b = 3 * NT
    big = [pltpu.make_async_copy(s_, d_, sems.at[b + i]) for i, (s_, d_) in enumerate(
        [(g_hbm, gm), (h_hbm, hm), (wm_hbm, wm), (w1_hbm, w1), (w2_hbm, w2)])]

    @pl.when(step == 0)
    def _conv():
        for cp in tile_copies(0):
            cp.start()
        dds[...] = dd_ref[...].astype(f32).reshape(1, D)

        @pl.loop(0, NT)
        def _tile(t):
            cs = pl.ds(pl.multiple_of(t * 128, 128), 128)
            for cp in tile_copies(t):
                cp.wait()

            @pl.when(t + 1 < NT)
            def _():
                for cp in tile_copies(t + 1):
                    cp.start()
            for i, tt in enumerate((0, 0, 1, 2, 3)):
                pl.when(t == tt)(big[i].start)
            taps = sk_ref[:, cs].astype(f32)
            tp = [jnp.broadcast_to(taps[i:i + 1], (32, 128)) for i in range(4)]
            skip = jnp.broadcast_to(dds[:, cs], (32, 128))
            for i in range(S // 128):
                st[i * 128:(i + 1) * 128, :] = sb[t, :, i * 128:(i + 1) * 128].T
            ku, vu, su = kb.at[t].bitcast(u32), vb.at[t].bitcast(u32), st.bitcast(u32)
            first = lax.broadcasted_iota(jnp.int32, (32, 128), 0) == 0

            def wrap(m):
                return [jnp.where(first, 0.0, pltpu.roll(z, 1, 0))
                        for z in _unpack(ku[pl.ds(m, 32, stride=32), :])]

            _, p1 = wrap(30)
            p2, p3 = wrap(31)

            def s1(it, carry):
                for u in range(U1):
                    m = it * U1 + u
                    p1, p2, p3 = carry
                    k0, k1 = _unpack(ku[pl.ds(m, 32, stride=32), :])
                    v0, v1 = _unpack(vu[pl.ds(m, 32, stride=32), :])
                    s0, s1_ = _unpack(su[pl.ds(m, 32, stride=32), :])
                    kv0 = ((k0 * tp[0] + p3 * tp[1] + p2 * tp[2] + p1 * tp[3]) * v0).astype(bf16)
                    kv1 = ((k1 * tp[0] + k0 * tp[1] + p3 * tp[2] + p2 * tp[3]) * v1).astype(bf16)
                    rhs = jnp.concatenate([kv0, kv1, s0.astype(bf16), s1_.astype(bf16)], axis=1)
                    r = _dot(f1_ref[...], rhs)
                    p = _pack(r[:32], r[32:])
                    a_kv[pl.ds(2 * m, 32, stride=65), :] = p[:, 0:128]
                    a_kv[pl.ds(2 * m + 1, 32, stride=65), :] = p[:, 128:256]
                    a_k[pl.ds(2 * m, 32, stride=65), :] = p[:, 256:384]
                    a_k[pl.ds(2 * m + 1, 32, stride=65), :] = p[:, 384:512]
                    kvs[m, 0] = kv0.astype(f32) * skip
                    kvs[m, 1] = kv1.astype(f32) * skip
                    carry = (p3, k0, k1)
                return carry

            s1(0, (p1, p2, p3))

            @pl.when(t == 0)
            def _():
                big[0].wait()
                big[1].wait()

            def freq(j, special):
                rows = pl.ds(j * 65, 64)
                rhs = jnp.concatenate([pltpu.bitcast(a_kv[rows, :], bf16),
                                       pltpu.bitcast(a_k[rows, :], bf16)], axis=1)
                x = _dot(gm[j], rhs)
                xr, xi, kr, ki = x[:64, :128], x[64:, :128], x[:64, 128:], x[64:, 128:]
                ii = xi * ki
                pr, pi = xr * kr - ii, xr * ki + xi * kr
                if special:
                    m0 = lax.broadcasted_iota(jnp.int32, (64, 128), 0) == 0
                    pr, pi = jnp.where(m0, xr * kr, pr), jnp.where(m0, ii, pi)
                z = _dot(hm[j], jnp.concatenate([pr, pi], axis=0).astype(bf16))
                bsc[pl.ds(j, 64, stride=33), :] = _pack(z[:64], z[64:])

            for j in range(U2):
                freq(j, j == 0)

            def s2(it, _):
                for u in range(U2):
                    freq(it * U2 + u, False)

            yu = y.at[t].bitcast(u32)

            def s3(it, _):
                for u in range(U3):
                    m = it * U3 + u
                    w = jnp.concatenate([bsc[pl.ds((2 * m + e) * 33, 32), :] for e in range(2)], axis=0)
                    rhs = jnp.concatenate([pltpu.bitcast(w[:32], bf16), pltpu.bitcast(w[32:], bf16)], axis=1)
                    r = _dot(fi_ref[...], rhs)
                    yu[pl.ds(m, 32, stride=32), :] = _pack(r[:, :128] + kvs[m, 0], r[:, 128:] + kvs[m, 1])

            s3(0, None)

        big[2].wait()
        c = c_ref[...].astype(f32)
        sc = jnp.broadcast_to(c * jax.nn.sigmoid(c), (16, D)).astype(bf16)
        mod[...] = _dot(sc, wm[...])
        big[3].wait()
        big[4].wait()

    sa, ca, ga, sb_, cb, gb = [mod[0:1, i * D:(i + 1) * D] for i in range(6)]
    b1 = b1_ref[...].astype(f32).reshape(1, F)
    b2 = b2_ref[...].astype(f32).reshape(1, D)
    for r in range(BM // SM):
        rows = pl.ds(pl.multiple_of(step * BM + r * SM, SM), SM)
        x = q_ref[r * SM:(r + 1) * SM, :].astype(f32)
        yy = jnp.concatenate([y[t, rows, :] for t in range(NT)], axis=1).astype(f32)
        x = x + ga * ((_ln(x) * (1 + ca) + sa) * yy)
        h = (_ln(x) * (1 + cb) + sb_).astype(bf16)
        o = b2
        for f0, f1 in zip(FS[:-1], FS[1:]):
            a = lax.dot_general(h, w1[f0:f1, :], (((1,), (1,)), ((), ())), preferred_element_type=f32)
            a = jax.nn.gelu(a + b1[:, f0:f1], approximate=True)
            o = o + _dot(a.astype(bf16), w2[f0:f1, :])
        o_ref[r * SM:(r + 1) * SM, :] = (x + gb * o).astype(o_ref.dtype)


@jax.jit
def pallas_adaLN_cond__ssm_conv_h3__dense_activation_gelu__prompt_kernel(
    A_q, A_k, A_v, A_shift_k, A_ssm_k, A_ssm_D, B_x, B_w1, B_b1, B_w2, B_b2, c, w_mod,
):
    del B_x
    full = lambda a: pl.BlockSpec(a.shape, lambda i: (0,) * a.ndim)
    small = [A_shift_k.T, A_ssm_D, B_b1, B_b2, c, _F1, _FI]
    hbm = [A_k.reshape(S, D), A_v.reshape(S, D), A_ssm_k, B_w1.T, B_w2, w_mod, _G, _H]
    V = pltpu.VMEM
    out = pl.pallas_call(
        _kernel,
        grid=(S // BM,),
        in_specs=[pl.BlockSpec((BM, D), lambda i: (i, 0))] + [full(a) for a in small]
        + [pl.BlockSpec(memory_space=pl.ANY)] * len(hbm),
        out_specs=pl.BlockSpec((BM, D), lambda i: (i, 0)),
        out_shape=jax.ShapeDtypeStruct((S, D), A_q.dtype),
        scratch_shapes=[
            V((NT, S, 128), bf16), V((NT, S, 128), bf16), V((NT, 128, S), bf16), V((S, 128), bf16),
            V((F, D), bf16), V((F, D), bf16), V((D, 6 * D), bf16),
            V((32, 128, 128), bf16), V((32, 128, 128), bf16),
            V((2600, 128), u32), V((2600, 128), u32), V((2600, 128), u32),
            V((32, 2, 32, 128), f32), V((NT, S, 128), bf16), V((16, 6 * D), f32), V((1, D), f32),
            pltpu.SemaphoreType.DMA((3 * NT + 5,)),
        ],
        compiler_params=pltpu.CompilerParams(
            dimension_semantics=("arbitrary",), vmem_limit_bytes=100 * 1024 * 1024),
    )(A_q.reshape(S, D), *small, *hbm)
    return out.reshape(1, S, D)
```

```python
import numpy as np
import jax
import jax.numpy as jnp
from jax import lax
import jax.experimental.pallas as pl
import jax.experimental.pallas.tpu as pltpu

S, D, F = 2048, 640, 1728
NT = D // 128
BM, SM = 512, 256
LAG = 4
L1 = 4
L3 = 8
FS = (0, 896, 1728)
U1, U2, U3 = 32, 32, 32


def _dft_consts():
    N = 4096
    n1 = np.arange(32)[None, :]
    j = np.arange(32)[:, None]
    a = 2 * np.pi * n1 * j / 64
    f1 = np.concatenate([np.cos(a), -np.sin(a)], 0)
    f1[32] = (-1.0) ** n1[0]
    n2 = np.arange(64)[None, :]
    k2 = np.arange(64)[:, None]
    G = np.zeros((32, 128, 128))
    H = np.zeros((32, 128, 128))
    for jj in range(1, 32):
        th = 2 * np.pi * ((n2 * (jj + 64 * k2)) % N) / N
        c, s = np.cos(th), np.sin(th)
        G[jj, :64, 0::2], G[jj, :64, 1::2] = c, s
        G[jj, 64:, 0::2], G[jj, 64:, 1::2] = -s, c
        H[jj, :64, :64], H[jj, :64, 64:] = c.T, -s.T
        H[jj, 64:, :64], H[jj, 64:, 64:] = s.T, c.T
    m = np.arange(32)[:, None]
    t0 = 2 * np.pi * ((n2 * m) % 64) / 64
    t1 = 2 * np.pi * ((n2 * (32 + 64 * m)) % N) / N
    r0, i0 = np.cos(t0), -np.sin(t0)
    i0[0] = (-1.0) ** n2[0]
    G[0, 0:32, 0::2], G[0, 64:96, 0::2] = r0, i0
    G[0, 32:64, 1::2], G[0, 96:128, 1::2] = np.cos(t1), -np.sin(t1)
    w = np.full((32, 1), 2.0)
    w[0] = 1.0
    H[0, :64, 0:32], H[0, :64, 64:96] = (w * r0).T, (w * i0).T
    H[0, 64:, 32:64], H[0, 64:, 96:128] = 2 * np.cos(t1).T, -2 * np.sin(t1).T
    a = a.T
    fi = np.zeros((32, 64))
    fi[:, 0::2], fi[:, 1::2] = 2 * np.cos(a), -2 * np.sin(a)
    fi[:, 0] = 1.0
    fi[:, 1] = (-1.0) ** np.arange(32)
    fi /= N
    f1, fi = np.kron(np.eye(4), f1), np.kron(np.eye(2), fi)
    bf = jnp.bfloat16
    return f1.astype(bf), G.astype(bf), H.astype(bf), fi.astype(bf)


_F1, _G, _H, _FI = _dft_consts()
f32, bf16, u32 = jnp.float32, jnp.bfloat16, jnp.uint32


def _unpack(u):
    lo = pltpu.bitcast(u << 16, f32)
    hi = pltpu.bitcast(u & jnp.uint32(0xFFFF0000), f32)
    return lo, hi


def _pack(lo, hi):
    return pltpu.pack_elementwise([lo, hi], packed_dtype=bf16)


def _dot(a, b):
    return jnp.dot(a, b, preferred_element_type=f32)


def _ln(x):
    m = jnp.mean(x, axis=-1, keepdims=True)
    xc = x - m
    v = jnp.mean(xc * xc, axis=-1, keepdims=True)
    return xc * lax.rsqrt(v + 1e-5)


def _kernel(q_ref, sk_ref, dd_ref, b1_ref, b2_ref, c_ref, f1_ref, fi_ref,
            k_hbm, v_hbm, s_hbm, w1_hbm, w2_hbm, wm_hbm, g_hbm, h_hbm,
            o_ref,
            kb, vb, sb, st, w1, w2, wm, gm, hm, a_kv, a_k, bsc, kvs, y, mod, dds, sems):
    step = pl.program_id(0)

    def tile_copies(t):
        cs = pl.ds(pl.multiple_of(t * 128, 128), 128)
        return (pltpu.make_async_copy(k_hbm.at[:, cs], kb.at[t], sems.at[3 * t]),
                pltpu.make_async_copy(v_hbm.at[:, cs], vb.at[t], sems.at[3 * t + 1]),
                pltpu.make_async_copy(s_hbm.at[cs, :], sb.at[t], sems.at[3 * t + 2]))

    b = 3 * NT
    big = [pltpu.make_async_copy(s_, d_, sems.at[b + i]) for i, (s_, d_) in enumerate(
        [(g_hbm, gm), (h_hbm, hm), (wm_hbm, wm), (w1_hbm, w1), (w2_hbm, w2)])]

    @pl.when(step == 0)
    def _conv():
        for cp in tile_copies(0):
            cp.start()
        dds[...] = dd_ref[...].astype(f32).reshape(1, D)

        @pl.loop(0, NT)
        def _tile(t):
            cs = pl.ds(pl.multiple_of(t * 128, 128), 128)
            for cp in tile_copies(t):
                cp.wait()

            @pl.when(t + 1 < NT)
            def _():
                for cp in tile_copies(t + 1):
                    cp.start()
            for i, tt in enumerate((0, 0, 1, 2, 3)):
                pl.when(t == tt)(big[i].start)
            taps = sk_ref[:, cs].astype(f32)
            tp = [jnp.broadcast_to(taps[i:i + 1], (32, 128)) for i in range(4)]
            skip = jnp.broadcast_to(dds[:, cs], (32, 128))
            for i in range(S // 128):
                st[i * 128:(i + 1) * 128, :] = sb[t, :, i * 128:(i + 1) * 128].T
            ku, vu, su = kb.at[t].bitcast(u32), vb.at[t].bitcast(u32), st.bitcast(u32)
            first = lax.broadcasted_iota(jnp.int32, (32, 128), 0) == 0

            def wrap(m):
                return [jnp.where(first, 0.0, pltpu.roll(z, 1, 0))
                        for z in _unpack(ku[pl.ds(m, 32, stride=32), :])]

            _, p1 = wrap(30)
            p2, p3 = wrap(31)

            def s1(it, carry):
                pend, grp = [], []
                for u in range(U1):
                    m = it * U1 + u
                    p1, p2, p3 = carry
                    k0, k1 = _unpack(ku[pl.ds(m, 32, stride=32), :])
                    v0, v1 = _unpack(vu[pl.ds(m, 32, stride=32), :])
                    s0, s1_ = _unpack(su[pl.ds(m, 32, stride=32), :])
                    kv0 = ((k0 * tp[0] + p3 * tp[1] + p2 * tp[2] + p1 * tp[3]) * v0).astype(bf16)
                    kv1 = ((k1 * tp[0] + k0 * tp[1] + p3 * tp[2] + p2 * tp[3]) * v1).astype(bf16)
                    rhs = jnp.concatenate([kv0, kv1, s0.astype(bf16), s1_.astype(bf16)], axis=1)
                    grp.append(rhs)
                    if len(grp) == 4:
                        r = _dot(f1_ref[...], jnp.concatenate(grp, axis=0))
                        grp.clear()
                        pend.extend((m - 3 + e, r[e * 64:(e + 1) * 64]) for e in range(4))
                    carry = (p3, k0, k1)
                    kvs[m, 0] = kv0.astype(f32) * skip
                    kvs[m, 1] = kv1.astype(f32) * skip
                    while len(pend) > L1:
                        st1(*pend.pop(0))
                for e in pend:
                    st1(*e)

            def st1(m, r):
                    p = _pack(r[:32], r[32:])
                    a_kv[pl.ds(2 * m, 32, stride=65), :] = p[:, 0:128]
                    a_kv[pl.ds(2 * m + 1, 32, stride=65), :] = p[:, 128:256]
                    a_k[pl.ds(2 * m, 32, stride=65), :] = p[:, 256:384]
                    a_k[pl.ds(2 * m + 1, 32, stride=65), :] = p[:, 384:512]

            s1(0, (p1, p2, p3))

            @pl.when(t == 0)
            def _():
                big[0].wait()
                big[1].wait()

            def fwd(j):
                rows = pl.ds(j * 65, 64)
                rhs = jnp.concatenate([pltpu.bitcast(a_kv[rows, :], bf16),
                                       pltpu.bitcast(a_k[rows, :], bf16)], axis=1)
                return _dot(gm[j], rhs)

            def mid(j, x):
                special = j == 0
                xr, xi, kr, ki = x[:64, :128], x[64:, :128], x[:64, 128:], x[64:, 128:]
                ii = xi * ki
                pr, pi = xr * kr - ii, xr * ki + xi * kr
                if special:
                    m0 = lax.broadcasted_iota(jnp.int32, (64, 128), 0) == 0
                    pr, pi = jnp.where(m0, xr * kr, pr), jnp.where(m0, ii, pi)
                return _dot(hm[j], jnp.concatenate([pr, pi], axis=0).astype(bf16))

            def put(j, z):
                bsc[pl.ds(j, 64, stride=33), :] = _pack(z[:64], z[64:])

            xs, zs = {}, {}
            for j in range(32 + 2 * LAG):
                if j < 32:
                    xs[j] = fwd(j)
                if 0 <= j - LAG < 32:
                    zs[j - LAG] = mid(j - LAG, xs.pop(j - LAG))
                if 0 <= j - 2 * LAG < 32:
                    put(j - 2 * LAG, zs.pop(j - 2 * LAG))
            yu = y.at[t].bitcast(u32)

            def s3(it, _):
                pend, grp = [], []
                for u in range(U3):
                    m = it * U3 + u
                    w = jnp.concatenate([bsc[pl.ds((2 * m + e) * 33, 32), :] for e in range(2)], axis=0)
                    rhs = jnp.concatenate([pltpu.bitcast(w[:32], bf16), pltpu.bitcast(w[32:], bf16)], axis=1)
                    grp.append(rhs)
                    if len(grp) == 2:
                        r = _dot(fi_ref[...], jnp.concatenate(grp, axis=0))
                        grp.clear()
                        pend.extend((m - 1 + e, r[e * 32:(e + 1) * 32]) for e in range(2))
                    while len(pend) > L3:
                        st3(*pend.pop(0))
                for e in pend:
                    st3(*e)

            def st3(m, r):
                    yu[pl.ds(m, 32, stride=32), :] = _pack(r[:, :128] + kvs[m, 0], r[:, 128:] + kvs[m, 1])

            s3(0, None)

        big[2].wait()
        c = c_ref[...].astype(f32)
        sc = jnp.broadcast_to(c * jax.nn.sigmoid(c), (16, D)).astype(bf16)
        mod[...] = _dot(sc, wm[...])
        big[3].wait()
        big[4].wait()

    sa, ca, ga, sb_, cb, gb = [mod[0:1, i * D:(i + 1) * D] for i in range(6)]
    b1 = b1_ref[...].astype(f32).reshape(1, F)
    b2 = b2_ref[...].astype(f32).reshape(1, D)
    for r in range(BM // SM):
        rows = pl.ds(pl.multiple_of(step * BM + r * SM, SM), SM)
        x = q_ref[r * SM:(r + 1) * SM, :].astype(f32)
        yy = jnp.concatenate([y[t, rows, :] for t in range(NT)], axis=1).astype(f32)
        x = x + ga * ((_ln(x) * (1 + ca) + sa) * yy)
        h = (_ln(x) * (1 + cb) + sb_).astype(bf16)
        o = b2
        for f0, f1 in zip(FS[:-1], FS[1:]):
            a = lax.dot_general(h, w1[f0:f1, :], (((1,), (1,)), ((), ())), preferred_element_type=f32)
            a = jax.nn.gelu(a + b1[:, f0:f1], approximate=True)
            o = o + _dot(a.astype(bf16), w2[f0:f1, :])
        o_ref[r * SM:(r + 1) * SM, :] = (x + gb * o).astype(o_ref.dtype)


@jax.jit
def pallas_adaLN_cond__ssm_conv_h3__dense_activation_gelu__prompt_kernel(
    A_q, A_k, A_v, A_shift_k, A_ssm_k, A_ssm_D, B_x, B_w1, B_b1, B_w2, B_b2, c, w_mod,
):
    del B_x
    full = lambda a: pl.BlockSpec(a.shape, lambda i: (0,) * a.ndim)
    small = [A_shift_k.T, A_ssm_D, B_b1, B_b2, c, _F1, _FI]
    hbm = [A_k.reshape(S, D), A_v.reshape(S, D), A_ssm_k, B_w1.T, B_w2, w_mod, _G, _H]
    V = pltpu.VMEM
    out = pl.pallas_call(
        _kernel,
        grid=(S // BM,),
        in_specs=[pl.BlockSpec((BM, D), lambda i: (i, 0))] + [full(a) for a in small]
        + [pl.BlockSpec(memory_space=pl.ANY)] * len(hbm),
        out_specs=pl.BlockSpec((BM, D), lambda i: (i, 0)),
        out_shape=jax.ShapeDtypeStruct((S, D), A_q.dtype),
        scratch_shapes=[
            V((NT, S, 128), bf16), V((NT, S, 128), bf16), V((NT, 128, S), bf16), V((S, 128), bf16),
            V((F, D), bf16), V((F, D), bf16), V((D, 6 * D), bf16),
            V((32, 128, 128), bf16), V((32, 128, 128), bf16),
            V((2600, 128), u32), V((2600, 128), u32), V((2600, 128), u32),
            V((32, 2, 32, 128), f32), V((NT, S, 128), bf16), V((16, 6 * D), f32), V((1, D), f32),
            pltpu.SemaphoreType.DMA((3 * NT + 5,)),
        ],
        compiler_params=pltpu.CompilerParams(
            dimension_semantics=("arbitrary",), vmem_limit_bytes=100 * 1024 * 1024),
    )(A_q.reshape(S, D), *small, *hbm)
    return out.reshape(1, S, D)
```

```python
import numpy as np
import jax
import jax.numpy as jnp
from jax import lax
import jax.experimental.pallas as pl
import jax.experimental.pallas.tpu as pltpu

S, D, F = 2048, 640, 1728
NT = D // 128
BM, SM = 512, 256
LAG = 3
L1 = 2
L3 = 4
FS = (0, 896, 1728)


def _dft_consts():
    N = 4096
    n1 = np.arange(32)[None, :]
    j = np.arange(32)[:, None]
    a = 2 * np.pi * n1 * j / 64
    f1 = np.concatenate([np.cos(a), -np.sin(a)], 0)
    f1[32] = (-1.0) ** n1[0]
    n2 = np.arange(64)[None, :]
    k2 = np.arange(64)[:, None]
    G = np.zeros((32, 128, 128))
    H = np.zeros((32, 128, 128))
    for jj in range(1, 32):
        th = 2 * np.pi * ((n2 * (jj + 64 * k2)) % N) / N
        c, s = np.cos(th), np.sin(th)
        G[jj, :64, 0::2], G[jj, :64, 1::2] = c, s
        G[jj, 64:, 0::2], G[jj, 64:, 1::2] = -s, c
        H[jj, :64, :64], H[jj, :64, 64:] = c.T, -s.T
        H[jj, 64:, :64], H[jj, 64:, 64:] = s.T, c.T
    m = np.arange(32)[:, None]
    t0 = 2 * np.pi * ((n2 * m) % 64) / 64
    t1 = 2 * np.pi * ((n2 * (32 + 64 * m)) % N) / N
    r0, i0 = np.cos(t0), -np.sin(t0)
    i0[0] = (-1.0) ** n2[0]
    G[0, 0:32, 0::2], G[0, 64:96, 0::2] = r0, i0
    G[0, 32:64, 1::2], G[0, 96:128, 1::2] = np.cos(t1), -np.sin(t1)
    w = np.full((32, 1), 2.0)
    w[0] = 1.0
    H[0, :64, 0:32], H[0, :64, 64:96] = (w * r0).T, (w * i0).T
    H[0, 64:, 32:64], H[0, 64:, 96:128] = 2 * np.cos(t1).T, -2 * np.sin(t1).T
    a = a.T
    fi = np.zeros((32, 64))
    fi[:, 0::2], fi[:, 1::2] = 2 * np.cos(a), -2 * np.sin(a)
    fi[:, 0] = 1.0
    fi[:, 1] = (-1.0) ** np.arange(32)
    fi /= N
    f1p = np.zeros((128, 64))
    f1p[:64, 0::2], f1p[64:, 1::2] = f1, f1
    f1, fi = np.kron(np.eye(2), f1p), np.kron(np.eye(2), fi)
    bf = jnp.bfloat16
    return f1.astype(bf), G.astype(bf), H.astype(bf), fi.astype(bf)


_F1, _G, _H, _FI = _dft_consts()
f32, bf16, u32 = jnp.float32, jnp.bfloat16, jnp.uint32


def _unpack(u):
    lo = pltpu.bitcast(u << 16, f32)
    hi = pltpu.bitcast(u & jnp.uint32(0xFFFF0000), f32)
    return lo, hi


def _pack(lo, hi):
    return pltpu.pack_elementwise([lo, hi], packed_dtype=bf16)


def _dot(a, b):
    return jnp.dot(a, b, preferred_element_type=f32)


def _ln(x):
    m = jnp.mean(x, axis=-1, keepdims=True)
    xc = x - m
    v = jnp.mean(xc * xc, axis=-1, keepdims=True)
    return xc * lax.rsqrt(v + 1e-5)


def _kernel(q_ref, sk_ref, dd_ref, b1_ref, b2_ref, c_ref, f1_ref, fi_ref,
            k_hbm, v_hbm, s_hbm, w1_hbm, w2_hbm, wm_hbm, g_hbm, h_hbm,
            o_ref,
            kb, vb, sb, w1, w2, wm, gm, hm, sts, akv, ak, bscs, y, mod, dds, sems):
    step = pl.program_id(0)

    def tile_copies(t):
        cs = pl.ds(pl.multiple_of(t * 128, 128), 128)
        return (pltpu.make_async_copy(k_hbm.at[:, cs], kb.at[t], sems.at[3 * t]),
                pltpu.make_async_copy(v_hbm.at[:, cs], vb.at[t], sems.at[3 * t + 1]),
                pltpu.make_async_copy(s_hbm.at[cs, :], sb.at[t], sems.at[3 * t + 2]))

    b = 3 * NT
    big = [pltpu.make_async_copy(s_, d_, sems.at[b + i]) for i, (s_, d_) in enumerate(
        [(g_hbm, gm), (h_hbm, hm), (wm_hbm, wm), (w1_hbm, w1), (w2_hbm, w2)])]

    @pl.when(step == 0)
    def _conv():
        for cp in tile_copies(0):
            cp.start()
        dds[...] = dd_ref[...].astype(f32).reshape(1, D)

        first = lax.broadcasted_iota(jnp.int32, (32, 128), 0) == 0
        m0 = lax.broadcasted_iota(jnp.int32, (64, 128), 0) == 0

        def stage1(t):
            cs = slice(t * 128, (t + 1) * 128)
            a_kv, a_k, st = akv[t % 2], ak[t % 2], sts[t % 2]
            for cp in tile_copies(t):
                cp.wait()
            if t + 1 < NT:
                for cp in tile_copies(t + 1):
                    cp.start()
            for i, tt in enumerate((0,0,3,1,2)):
                if t == tt:
                    big[i].start()
            taps = sk_ref[:, cs].astype(f32)
            tp = [jnp.broadcast_to(taps[i:i + 1], (32, 128)) for i in range(4)]
            for i in range(S // 128):
                st[i * 128:(i + 1) * 128, :] = sb[t, :, i * 128:(i + 1) * 128].T
            ku, vu, su = kb.at[t].bitcast(u32), vb.at[t].bitcast(u32), st.bitcast(u32)

            def wrap(m):
                return [jnp.where(first, 0.0, pltpu.roll(z, 1, 0))
                        for z in _unpack(ku[pl.ds(m, 32, stride=32), :])]

            _, p1 = wrap(30)
            p2, p3 = wrap(31)
            pend, grp = [], []

            def put(m, r):
                for e in range(2):
                    p = _pack(r[e * 64:e * 64 + 32], r[e * 64 + 32:e * 64 + 64])
                    a_kv[pl.ds(2 * m + e, 32, stride=65), :] = p[:, :128]
                    a_k[pl.ds(2 * m + e, 32, stride=65), :] = p[:, 128:]

            for m in range(32):
                k0, k1 = _unpack(ku[pl.ds(m, 32, stride=32), :])
                v0, v1 = _unpack(vu[pl.ds(m, 32, stride=32), :])
                kv0 = (k0 * tp[0] + p3 * tp[1] + p2 * tp[2] + p1 * tp[3]) * v0
                kv1 = (k1 * tp[0] + k0 * tp[1] + p3 * tp[2] + p2 * tp[3]) * v1
                p1, p2, p3 = p3, k0, k1
                grp.append(jnp.concatenate([pltpu.bitcast(_pack(kv0, kv1), bf16),
                                            pltpu.bitcast(su[pl.ds(m, 32, stride=32), :], bf16)], axis=1))
                if len(grp) == 2:
                    r = _dot(f1_ref[...], jnp.concatenate(grp, axis=0))
                    grp.clear()
                    pend.extend([(m - 1, r[:128]), (m, r[128:])])
                while len(pend) > L1 or (pend and m == 31):
                    put(*pend.pop(0))
                yield

        def stage2(t):
            a_kv, a_k, bsc = akv[t % 2], ak[t % 2], bscs[t % 2]
            if t == 0:
                big[0].wait()
                big[1].wait()
            skip = dds[:, t * 128:(t + 1) * 128]
            xs, zs = {}, {}
            for j in range(32 + 2 * LAG):
                if j < 32:
                    rows = pl.ds(j * 65, 64)
                    xs[j] = _dot(gm[j], jnp.concatenate(
                        [pltpu.bitcast(a_kv[rows, :], bf16), pltpu.bitcast(a_k[rows, :], bf16)], axis=1))
                if 0 <= j - LAG < 32:
                    x = xs.pop(j - LAG)
                    xr, xi, kr, ki = x[:64, :128], x[64:, :128], x[:64, 128:] + skip, x[64:, 128:]
                    if j == LAG:
                        ii = xi * jnp.where(m0, ki + skip, ki)
                        pr, pi = jnp.where(m0, xr * kr, xr * kr - ii), jnp.where(m0, ii, xr * ki + xi * kr)
                    else:
                        pr, pi = xr * kr - xi * ki, xr * ki + xi * kr
                    zs[j - LAG] = _dot(hm[j - LAG], jnp.concatenate([pr, pi], axis=0).astype(bf16))
                if 0 <= j - 2 * LAG < 32:
                    z = zs.pop(j - 2 * LAG)
                    bsc[pl.ds(j - 2 * LAG, 64, stride=33), :] = _pack(z[:64], z[64:])
                if j < 31:
                    yield
            yield

        def stage3(t):
            bsc, yu = bscs[t % 2], y.at[t].bitcast(u32)
            pend, grp = [], []
            for m in range(32):
                grp.append(jnp.concatenate(
                    [pltpu.bitcast(bsc[pl.ds((2 * m + e) * 33, 32), :], bf16) for e in range(2)], axis=1))
                if len(grp) == 2:
                    r = _dot(fi_ref[...], jnp.concatenate(grp, axis=0))
                    grp.clear()
                    pend.extend([(m - 1, r[:32]), (m, r[32:])])
                while len(pend) > L3 or (pend and m == 31):
                    mm, r = pend.pop(0)
                    yu[pl.ds(mm, 32, stride=32), :] = _pack(r[:, :128], r[:, 128:])
                yield

        for i in range(NT + 2):
            gens = [g(t) for g, t in ((stage2, i - 1), (stage1, i), (stage3, i - 2)) if 0 <= t < NT]
            for _ in range(32):
                for g in gens:
                    next(g)

        big[2].wait()
        c = c_ref[...].astype(f32)
        sc = jnp.broadcast_to(c * jax.nn.sigmoid(c), (16, D)).astype(bf16)
        mod[...] = _dot(sc, wm[...])
        big[3].wait()
        big[4].wait()

    sa, ca, ga, sb_, cb, gb = [mod[0:1, i * D:(i + 1) * D] for i in range(6)]
    b1 = b1_ref[...].astype(f32).reshape(1, F)
    b2 = b2_ref[...].astype(f32).reshape(1, D)
    for r in range(BM // SM):
        rows = pl.ds(pl.multiple_of(step * BM + r * SM, SM), SM)
        x = q_ref[r * SM:(r + 1) * SM, :].astype(f32)
        yy = jnp.concatenate([y[t, rows, :] for t in range(NT)], axis=1).astype(f32)
        x = x + ga * ((_ln(x) * (1 + ca) + sa) * yy)
        h = (_ln(x) * (1 + cb) + sb_).astype(bf16)
        o = b2
        for f0, f1 in zip(FS[:-1], FS[1:]):
            a = lax.dot_general(h, w1[f0:f1, :], (((1,), (1,)), ((), ())), preferred_element_type=f32)
            a = jax.nn.gelu(a + b1[:, f0:f1], approximate=True)
            o = o + _dot(a.astype(bf16), w2[f0:f1, :])
        o_ref[r * SM:(r + 1) * SM, :] = (x + gb * o).astype(o_ref.dtype)


@jax.jit
def pallas_adaLN_cond__ssm_conv_h3__dense_activation_gelu__prompt_kernel(
    A_q, A_k, A_v, A_shift_k, A_ssm_k, A_ssm_D, B_x, B_w1, B_b1, B_w2, B_b2, c, w_mod,
):
    del B_x
    full = lambda a: pl.BlockSpec(a.shape, lambda i: (0,) * a.ndim)
    small = [A_shift_k.T, A_ssm_D, B_b1, B_b2, c, _F1, _FI]
    hbm = [A_k.reshape(S, D), A_v.reshape(S, D), A_ssm_k, B_w1.T, B_w2, w_mod, _G, _H]
    V = pltpu.VMEM
    out = pl.pallas_call(
        _kernel,
        grid=(S // BM,),
        in_specs=[pl.BlockSpec((BM, D), lambda i: (i, 0))] + [full(a) for a in small]
        + [pl.BlockSpec(memory_space=pl.ANY)] * len(hbm),
        out_specs=pl.BlockSpec((BM, D), lambda i: (i, 0)),
        out_shape=jax.ShapeDtypeStruct((S, D), A_q.dtype),
        scratch_shapes=[
            V((NT, S, 128), bf16), V((NT, S, 128), bf16), V((NT, 128, S), bf16),
            V((F, D), bf16), V((F, D), bf16), V((D, 6 * D), bf16),
            V((32, 128, 128), bf16), V((32, 128, 128), bf16),
            [V((S, 128), bf16)] * 2, [V((2080, 128), u32)] * 2, [V((2080, 128), u32)] * 2,
            [V((2112, 128), u32)] * 2, V((NT, S, 128), bf16), V((16, 6 * D), f32), V((1, D), f32),
            pltpu.SemaphoreType.DMA((3 * NT + 5,)),
        ],
        compiler_params=pltpu.CompilerParams(
            dimension_semantics=("arbitrary",), vmem_limit_bytes=100 * 1024 * 1024),
    )(A_q.reshape(S, D), *small, *hbm)
    return out.reshape(1, S, D)
```
